```python
import os as _os
_os.environ.setdefault("JAX_PLATFORMS", "cpu")
import jax
import jax.numpy as jnp

def _softmax(x, axis=-1):
    return jax.nn.softmax(x, axis=axis)
def _gelu(x):
    return jax.nn.gelu(x, approximate=True)
def _silu(x):
    return jax.nn.silu(x)
def _sigmoid(x):
    return jax.nn.sigmoid(x)
def _layernorm(x, axis=-1, eps=1e-5):
    m = jnp.mean(x, axis=axis, keepdims=True)
    v = jnp.var(x, axis=axis, keepdims=True)
    return (x - m) / jnp.sqrt(v + eps)
def _scatter_add(tgt, idx, src, axis=0):
    return tgt.at[idx].add(src)
def _segment_sum(src, seg, n):
    return jax.ops.segment_sum(src, seg, n)
class _Rng:
    def __init__(self, key):
        self._k = key
    def _next(self):
        self._k, sub = jax.random.split(self._k)
        return sub
    def normal(self, shape):
        return jax.random.normal(self._next(), shape, dtype=jnp.bfloat16)
    def randint(self, lo, hi, shape):
        return jax.random.randint(self._next(), shape, lo, hi, dtype=jnp.int32)
    def uniform(self, shape, lo=0.0, hi=1.0):
        return jax.random.uniform(self._next(), shape, jnp.bfloat16, lo, hi)
    def permutation(self, n):
        return jax.random.permutation(self._next(), n)


kernel_name = 'interleave_layers__sliding_local_dilated__moe_arch_mod__prompt'

def setup_inputs():
    _rng = _Rng(jax.random.key(int.from_bytes(__import__("os").urandom(4), "little")))
    _w = (lambda a: (lambda t: t.astype(jnp.bfloat16) if jnp.issubdtype(t.dtype, jnp.floating) else t)(jnp.asarray(a)))
    def _A_setup():
        B, S, D = 1, 2048, 512
        return {
            "x": _w((lambda *s: _rng.normal(s) * 0.05)(B, S, D)),
            "wqkv": _w((lambda *s: _rng.normal(s) * 0.05)(D, 3 * D)),
            "wo": _w((lambda *s: _rng.normal(s) * 0.05)(D, D)),
        }
    _A_in = _A_setup()

    def _B_setup():
        B, S, D, F, C = 1, 2048, 512, 1376, 2
        return {
            "x": _w((lambda *s: _rng.normal(s) * 0.05)(B, S, D)),
            "w_r": _w((lambda *s: _rng.normal(s) * 0.05)(D)),
            "w_gate": _w((lambda *s: _rng.normal(s) * 0.05)(D, F)),
            "w_up": _w((lambda *s: _rng.normal(s) * 0.05)(D, F)),
            "w_down": _w((lambda *s: _rng.normal(s) * 0.05)(F, D)),
        }
    _B_in = _B_setup()

    return {
        "A_x": _A_in["x"],
        "A_wqkv": _A_in["wqkv"],
        "A_wo": _A_in["wo"],
        "B_x": _B_in["x"],
        "B_w_r": _B_in["w_r"],
        "B_w_gate": _B_in["w_gate"],
        "B_w_up": _B_in["w_up"],
        "B_w_down": _B_in["w_down"],
    }

def reference(A_x, A_wqkv, A_wo, B_x, B_w_r, B_w_gate, B_w_up, B_w_down):
    def _A_ref(x, wqkv, wo):
        B, S, D = x.shape
        H = 32; Dh = D // H
        W, dil = 8, 2
        qkv = (lambda x, *d: x.transpose(*d))((x @ wqkv).reshape(B, S, 3, H, Dh), 2, 0, 3, 1, 4)
        q, k, v = qkv[0], qkv[1], qkv[2]
        scale = Dh ** -0.5
        pos = jnp.arange(S)
        off = jnp.arange(W) * dil
        idx = pos[:, None] - off[None, :]
        mask = idx >= 0
        idx_c = jnp.where(mask, idx, 0).reshape(-1)
        kg = k[:, :, idx_c, :].reshape(B, H, S, W, Dh)
        vg = v[:, :, idx_c, :].reshape(B, H, S, W, Dh)
        logits = jnp.einsum("bhsd,bhswd->bhsw", q, kg) * scale
        logits = jnp.where(mask[None, None, :, :], logits, -1e9)
        attn = _softmax(logits, axis=-1)
        o = jnp.einsum("bhsw,bhswd->bhsd", attn, vg)
        return (lambda x, *d: x.transpose(*d))(o, 0, 2, 1, 3).reshape(B, S, D) @ wo

    def _B_ref(x, w_r, w_gate, w_up, w_down):
        B, S, D = x.shape
        C = 2
        r = x @ w_r
        idx = jnp.argsort(-r, axis=-1)[:, :C]
        idx_e = jnp.repeat(idx.reshape(B, C, 1), D, axis=2)
        x_sel = jnp.take_along_axis(x, idx_e, axis=1)
        g = _silu(x_sel @ w_gate)
        u = x_sel @ w_up
        y = (g * u) @ w_down
        r_sel = _sigmoid(jnp.take_along_axis(r, idx, axis=1))
        y = y * r_sel.reshape(B, C, 1)
        b_off = (jnp.arange(B) * S).reshape(B, 1)
        flat_idx = (idx + b_off).reshape(B * C)
        zero = (x * 0.0).reshape(B * S, D)
        upd = _scatter_add(zero, flat_idx, y.reshape(B * C, D), axis=0)
        return x + upd.reshape(B, S, D)

    x = A_x
    x = x + _A_ref(_layernorm(x, axis=-1), A_wqkv, A_wo)
    x = x + _B_ref(_layernorm(x, axis=-1), B_w_r, B_w_gate, B_w_up, B_w_down)
    x = x + _A_ref(_layernorm(x, axis=-1), A_wqkv, A_wo)
    x = x + _B_ref(_layernorm(x, axis=-1), B_w_r, B_w_gate, B_w_up, B_w_down)
    return x
```

```python
import jax
import jax.numpy as jnp
from jax import lax
import jax.experimental.pallas as pl
import jax.experimental.pallas.tpu as pltpu

S, D, F = 2048, 512, 1376
NB = 16
EPS = 1e-5
f32 = jnp.float32
bf16 = jnp.bfloat16
NT = (((1,), (1,)), ((), ()))


def _ln(x):
    m = jnp.mean(x, axis=0, keepdims=True)
    d = x - m
    v = jnp.mean(d * d, axis=0, keepdims=True)
    return d * lax.rsqrt(v + EPS)


def kernel(x_hbm, wqkv_hbm, wo_hbm, wr_ref, wg_hbm, wu_hbm, wd_hbm, out_hbm,
           xin, xT, wqkv_s, wT, wo_s, woT, q_s, kext, vext, o_s, r_s, wg, wu, wd, wrb, sems):
    cps = [
        None,
        pltpu.make_async_copy(wqkv_hbm, wqkv_s, sems.at[1]),
        pltpu.make_async_copy(wo_hbm, wo_s, sems.at[2]),
        pltpu.make_async_copy(wg_hbm, wg, sems.at[3]),
        pltpu.make_async_copy(wu_hbm, wu, sems.at[4]),
        pltpu.make_async_copy(wd_hbm, wd, sems.at[5]),
    ]
    xcp = [pltpu.make_async_copy(x_hbm.at[0, :, k * 128:(k + 1) * 128], xin.bitcast(bf16).at[k * S:(k + 1) * S], sems.at[0]) for k in range(4)]
    for c in xcp + cps[1:]:
        c.start()

    ri = lax.broadcasted_iota(jnp.int32, (128, 128), 0)
    ci = lax.broadcasted_iota(jnp.int32, (128, 128), 1)
    perm = jnp.where(ci == (ri % 8) * 16 + ri // 8, 1.0, 0.0).astype(bf16)

    wrb[...] = jnp.broadcast_to(wr_ref[...].astype(f32).reshape(1, D), (128, D)).T

    cps[1].wait()
    for b in range(12):
        t = lax.dot_general(perm, wqkv_s[:, b * 128:(b + 1) * 128], NT, preferred_element_type=f32)
        wT[b * 128:(b + 1) * 128, :] = t.astype(bf16)

    for c in xcp:
        c.wait()
    x32 = xin

    @pl.loop(0, NB)
    def _(n):
        j = n // 8
        c = n % 8
        for k in range(4):
            w = x32[pl.ds(k * 1024 + j * 512 + c, 64, stride=8), :]
            xb = pltpu.bitcast(w, bf16)
            xT[n, k * 128:(k + 1) * 128, :] = xb.astype(f32).T

    cps[2].wait()
    for b in range(4):
        t = jnp.dot(perm, wo_s[b * 128:(b + 1) * 128, :], preferred_element_type=f32)
        woT[:, b * 128:(b + 1) * 128] = t.T.astype(bf16)

    lane = lax.broadcasted_iota(jnp.int32, (8, 128), 1)
    laneD = lax.broadcasted_iota(jnp.int32, (D, 128), 1)

    @pl.loop(0, 2)
    def _(layer):
        @pl.loop(0, NB)
        def _(n):
            j = n // 8
            c = n % 8
            h = _ln(xT[n]).astype(bf16)
            q_s[n] = jnp.dot(wT[0:D, :], h, preferred_element_type=f32) * 0.25
            kext[j, c + 7] = jnp.dot(wT[D:2 * D, :], h, preferred_element_type=f32)
            vext[j, c + 7] = jnp.dot(wT[2 * D:3 * D, :], h, preferred_element_type=f32)

        v0 = jnp.broadcast_to(vext[0, 7][:, 0:1], (D, 128))

        @pl.loop(1, 8)
        def _(c):
            k0 = pltpu.roll(kext[0, c + 7], 2, 1)
            k1 = pltpu.roll(kext[1, c + 7], 2, 1)
            kext[0, c - 1] = k0
            kext[1, c - 1] = jnp.where(laneD < 2, k0, k1)
            va = pltpu.roll(vext[0, c + 7], 2, 1)
            vb = pltpu.roll(vext[1, c + 7], 2, 1)
            vext[0, c - 1] = jnp.where(laneD < 2, v0, va)
            vext[1, c - 1] = jnp.where(laneD < 2, va, vb)

        @pl.loop(0, NB)
        def _(n):
            j = n // 8
            c = n % 8
            for g in range(4):
                ls = []
                for w in range(8):
                    e = c + 7 - w
                    acc = None
                    for d in range(16):
                        rows = pl.ds(g * 128 + d * 8, 8)
                        t = q_s[n, rows, :] * kext[j, e, rows, :]
                        acc = t if acc is None else acc + t
                    if w > 0:
                        lim = jnp.where((j == 0) & (c < w), 2, 0)
                        acc = jnp.where(lane < lim, -1e9, acc)
                    ls.append(acc)
                m = ls[0]
                for w in range(1, 8):
                    m = jnp.maximum(m, ls[w])
                es = [jnp.exp(l - m) for l in ls]
                s = es[0]
                for w in range(1, 8):
                    s = s + es[w]
                inv = 1.0 / s
                ps = [e_ * inv for e_ in es]
                for d2 in range(8):
                    outs = []
                    for d in (2 * d2, 2 * d2 + 1):
                        rows = pl.ds(g * 128 + d * 8, 8)
                        acc = None
                        for w in range(8):
                            t = ps[w] * vext[j, c + 7 - w, rows, :]
                            acc = t if acc is None else acc + t
                        outs.append(acc)
                    o_s[n, pl.ds(g * 128 + d2 * 16, 16), :] = jnp.concatenate(outs, axis=0).astype(bf16)

        @pl.loop(0, NB)
        def _(n):
            x1 = xT[n] + jnp.dot(woT[...], o_s[n], preferred_element_type=f32)
            h = _ln(x1)
            r_s[pl.ds(n, 1), :] = jnp.sum(h * wrb[...], axis=0, keepdims=True)
            xT[n] = x1 + h
            o_s[n] = h.astype(bf16)

        @pl.when(layer == 0)
        def _():
            cps[3].wait()
            cps[4].wait()
            cps[5].wait()

        r = r_s[...]
        rn = lax.broadcasted_iota(jnp.int32, (NB, 128), 0)
        rl = lax.broadcasted_iota(jnp.int32, (NB, 128), 1)
        pos = (rn // 8) * 1024 + (rl // 2) * 16 + (rn % 8) * 2 + rl % 2
        big = jnp.int32(1 << 20)
        m1 = jnp.max(r)
        p1 = jnp.min(jnp.where(r == m1, pos, big))
        rr = jnp.where(pos == p1, -jnp.inf, r)
        m2 = jnp.max(rr)
        p2 = jnp.min(jnp.where((rr == m2) & (pos != p1), pos, big))
        sel = []
        xs = None
        row8 = lax.broadcasted_iota(jnp.int32, (16, 128), 0)
        lane8 = lax.broadcasted_iota(jnp.int32, (16, 128), 1)
        for t, p in enumerate((p1, p2)):
            p = jnp.minimum(p, S - 1)
            nblk = (p // 1024) * 8 + (p % 16) // 2
            ln_ = ((p % 1024) // 16) * 2 + p % 2
            oh = jnp.where((row8 == t) & (lane8 == ln_), 1.0, 0.0).astype(bf16)
            part = lax.dot_general(oh, o_s[nblk], NT, preferred_element_type=f32)
            xs = part if xs is None else xs + part
            sel.append((nblk, oh))
        xs = xs.astype(bf16)
        g_ = lax.dot_general(xs, wg[...], NT, preferred_element_type=f32)
        u_ = lax.dot_general(xs, wu[...], NT, preferred_element_type=f32)
        act = (g_ * jax.nn.sigmoid(g_) * u_).astype(bf16)
        y = jnp.dot(act, wd[...], preferred_element_type=f32)
        rowD = lax.broadcasted_iota(jnp.int32, (16, D), 0)
        y = y * jax.nn.sigmoid(jnp.where(rowD == 0, m1, m2))
        yh = y.astype(bf16)
        for nblk, oh in sel:
            upd = lax.dot_general(yh, oh, (((0,), (0,)), ((), ())), preferred_element_type=f32)
            xT[nblk] = xT[nblk] + upd

    @pl.loop(0, NB)
    def _(n):
        j = n // 8
        c = n % 8
        for k in range(4):
            xb = xT[n, k * 128:(k + 1) * 128, :].T.astype(bf16)
            x32[pl.ds(k * 1024 + j * 512 + c, 64, stride=8), :] = pltpu.bitcast(xb, jnp.uint32)

    ocp = [pltpu.make_async_copy(xin.bitcast(bf16).at[k * S:(k + 1) * S], out_hbm.at[0, :, k * 128:(k + 1) * 128], sems.at[6]) for k in range(4)]
    for c in ocp:
        c.start()
    for c in ocp:
        c.wait()


@jax.jit
def pallas_interleave_layers__sliding_local_dilated__moe_arch_mod__prompt_kernel(
    A_x, A_wqkv, A_wo, B_x, B_w_r, B_w_gate, B_w_up, B_w_down):
    any_ = pl.BlockSpec(memory_space=pltpu.MemorySpace.HBM)
    return pl.pallas_call(
        kernel,
        out_shape=jax.ShapeDtypeStruct((1, S, D), bf16),
        in_specs=[any_, any_, any_, pl.BlockSpec(memory_space=pltpu.VMEM), any_, any_, any_],
        out_specs=any_,
        scratch_shapes=[
            pltpu.VMEM((4 * S // 2 + 8, 128), jnp.uint32),
            pltpu.VMEM((NB, D, 128), f32),
            pltpu.VMEM((D, 3 * D), bf16),
            pltpu.VMEM((3 * D, D), bf16),
            pltpu.VMEM((D, D), bf16),
            pltpu.VMEM((D, D), bf16),
            pltpu.VMEM((NB, D, 128), f32),
            pltpu.VMEM((2, 15, D, 128), f32),
            pltpu.VMEM((2, 15, D, 128), f32),
            pltpu.VMEM((NB, D, 128), bf16),
            pltpu.VMEM((NB, 128), f32),
            pltpu.VMEM((F, D), bf16),
            pltpu.VMEM((F, D), bf16),
            pltpu.VMEM((F, D), bf16),
            pltpu.VMEM((D, 128), f32),
            pltpu.SemaphoreType.DMA((8,)),
        ],
        compiler_params=pltpu.CompilerParams(vmem_limit_bytes=100 * 1024 * 1024),
    )(A_x, A_wqkv, A_wo, B_w_r, B_w_gate.T, B_w_up.T, B_w_down)
```

```python
import jax
import jax.numpy as jnp
from jax import lax
import jax.experimental.pallas as pl
import jax.experimental.pallas.tpu as pltpu

S, D, F = 2048, 512, 1376
FP = 1408
NB = 16
EPS = 1e-5
SPARE = 40
f32 = jnp.float32
bf16 = jnp.bfloat16
u32 = jnp.uint32
i32 = jnp.int32
NT = (((1,), (1,)), ((), ()))
QA, PA, MA, TA, SLOTS = 0, 128, 144, 152, 168
PIECES = ((0, 2), (2, 2), (4, 2), (6, 2), (8, 8))
OUTS = ((0, 4), (4, 4), (8, 4), (12, 2), (14, 2))
PLAN = "p0 q9 p1 q10 p2 p3 q11 p8 p4 q12 p9 p5 q13 p6 q14 p10 p7 q15 p11 p12 p13 p14"
PREP, ATT, FIN, WPREP = 676, 2184, 256, 1280
DL = 24


def _tree(vals, op):
    vals = list(vals)
    while len(vals) > 1:
        vals = [op(vals[i], vals[i + 1]) for i in range(0, len(vals), 2)]
    return vals[0]


class _Acc:
    def __init__(self):
        self.a = [None, None]
        self.i = 0

    def add(self, t):
        k = self.i % 2
        self.a[k] = t if self.a[k] is None else self.a[k] + t
        self.i += 1

    def tile(self):
        return self.a[0] + self.a[1]


class _Pacer:
    def __init__(self):
        self.urgent, self.jobs, self.rate, self.credit = [], [], 0.0, 0.0

    def step(self):
        queue = self.urgent or self.jobs
        cost = next(queue[0], None)
        if cost is None:
            queue.pop(0)
        else:
            self.credit -= cost
        return cost != 0

    def until(self, done):
        while not done():
            if not self.step():
                raise ValueError("job traced before its operand")

    def drain(self):
        self.until(lambda: not (self.urgent or self.jobs))

    def set(self, jobs, cost=0, tiles=1):
        self.drain()
        self.jobs, self.rate, self.credit = list(jobs), cost / tiles, 0.0

    def run(self, tiles):
        self.credit += self.rate * tiles
        while (self.urgent or self.jobs) and self.credit > 0 and self.step():
            pass


def _rows(i):
    return pl.ds(i * 8, 8)


def _tile(v, i):
    return v[i * 8:(i + 1) * 8]


def _bc(v):
    return jnp.broadcast_to(v, (8, 128))


def _colsum(t):
    return jnp.sum(t, axis=0, keepdims=True)


def _as_bf16(w):
    return pltpu.bitcast(w, bf16)


def _as_u32(v):
    return pltpu.bitcast(v, u32)


def _bits_f32(w):
    return lax.bitcast_convert_type(w, f32)


def _bits_u32(v):
    return lax.bitcast_convert_type(v, u32)


def _lo(w):
    return _bits_f32(w << 16)


def _hi(w):
    return _bits_f32(w & u32(0xFFFF0000))


def _shift(t):
    return _colsum(t) * 0.125


def _moments(s1, s2):
    dm = _colsum(s1) * (1.0 / D)
    var = jnp.maximum(_colsum(s2) * (1.0 / D) - dm * dm, 0.0)
    return dm, lax.rsqrt(var + EPS)


def kernel(x_hbm, wqkv_hbm, wo_hbm, wr_hbm, wg_hbm, wu_hbm, wd_hbm, out_hbm,
           x0, x1, x2, x3, x4, wk0, wk1, wk2, wk3, raw_q, raw_v, raw_o, tmp_k, tmp_v, tmp_q,
           wT_q, wT_k, wT_v, wT_o, xb, k0, v0, xa0, h0, r_s, m_s, rs_s, sums,
           raw_g, raw_u, wd, wg, wu, wr_s, wrb, patch, st_a, st_b, st_c, sems):
    xs, raw_k = (x0, x1, x2, x3, x4), (wk0, wk1, wk2, wk3)
    lane = lax.broadcasted_iota(i32, (8, 128), 1)
    pacer, hv, ov, xa, q_ready = _Pacer(), {}, {}, {}, set()
    late, slow, marks, stage = [], [], [0], [st_a]

    def col_copies(src, nrows, col0, dst, pitch, sem):
        return [pltpu.make_async_copy(
            src.bitcast(u32).at[:, pl.ds(col0 + 128 * k, 128)],
            dst.at[pl.ds(k * pitch // 2, nrows // 2)], sem) for k in range(4)]

    def blocks_hbm(ref, first, n, k):
        return ref.bitcast(u32).at[pl.ds(64 * (first // 8), 64), pl.ds(first % 8, n), pl.ds(128 * k, 128)]

    def blocks_vmem(ref, first, n, k):
        return ref.reshape(ref.shape[0] // 8, 8, 128).at[pl.ds(64 * k, 64), pl.ds(first % 8, n), :]

    cp_x = [[pltpu.make_async_copy(blocks_hbm(x_hbm, *p, k), blocks_vmem(xs[q], *p, k), sems.at[q])
             for k in range(4)] for q, p in enumerate(PIECES)]
    cp_out = [[pltpu.make_async_copy(blocks_vmem(xs[q], *p, k), blocks_hbm(out_hbm, *p, k), sems.at[q])
               for k in range(4)] for q, p in enumerate(OUTS)]
    cp_k = [pltpu.make_async_copy(wqkv_hbm.bitcast(u32).at[:, pl.ds(D + 128 * g, 128)],
                                  raw_k[g].at[pl.ds(0, D // 2)], sems.at[5 + g]) for g in range(4)]
    cp_q = col_copies(wqkv_hbm, D, 0, raw_q, D, sems.at[9])
    cp_v = col_copies(wqkv_hbm, D, 2 * D, raw_v, D, sems.at[10])
    cp_o = col_copies(wo_hbm, D, 0, raw_o, D, sems.at[11])
    cp_g = col_copies(wg_hbm, F, 0, raw_g, FP, sems.at[12])
    cp_u = col_copies(wu_hbm, F, 0, raw_u, FP, sems.at[13])
    cp_d = col_copies(wd_hbm, F, 0, wd, FP, sems.at[14])
    cp_r = [pltpu.make_async_copy(wr_hbm, wr_s, sems.at[15])]

    def start(cps):
        for c in cps:
            c.start()

    def wait(cps):
        for c in cps:
            c.wait()

    for ref in (raw_g, raw_u, wd):
        for k in range(4):
            ref[pl.ds(k * (FP // 2) + F // 2, (FP - F) // 2), :] = jnp.zeros(((FP - F) // 2, 128), u32)
    for cps in (cp_r, cp_x[0], cp_k, cp_x[1], cp_x[2], cp_x[3], cp_v):
        start(cps)

    @pl.when(pl.program_id(0) == 0)
    def _():
        wait(cp_r)
        wait(cp_x[0])
    wr = wr_s[...].astype(f32).reshape(1, D)

    zeros = (jnp.abs(wr[:, 0:128]) < 0.0).astype(i32)
    z0, z1 = zeros[0, 0], zeros[0, 1]

    def put(i, v):
        stage[0][i] = v

    def get(i):
        return stage[0][i + z0]

    def mark(v):
        marks[0] += 1
        stage[0][TA + marks[0] % 8 + z1] = v

    def later(action, delay=DL):
        while len(slow) <= delay:
            slow.append([])
        slow[delay].append(action)

    def mark_later(w, delay=DL):
        later(lambda: mark(_bits_f32(_tile(w, w.shape[0] // 8 - 1))), delay)

    def settle():
        pacer.drain()
        while slow:
            for action in slow.pop(0):
                action()
        late.clear()

    def switch(buf):
        settle()
        stage[0] = buf
        put(MA + 7, jnp.zeros((8, 128), f32))

    def spare(ref, z, slot):
        return ref.at[pl.ds(ref.shape[0] - SPARE + (slot + z) * 8, 8)]

    def wait_here(cps, ref, slot=0):
        spare(ref, z1, slot)[...] = _bits_u32(get(MA + 7))
        wait(cps)

    def start_here(cps, ref):
        spare(ref, z1, 1)[...] = _bits_u32(get(MA + 7))
        start(cps)
        spare(ref, z1, 2)[...] = jnp.zeros((8, 128), u32)
        mark(_bits_f32(spare(ref, z0, 2)[...]))

    def mm(w, rhs, sink, marked=True, riders=None, m=64, tiles=range(64)):
        for i in tiles:
            if i % m == 0:
                lhs = jnp.concatenate([_as_bf16(w[k, pl.ds(i * 4, m * 4), :]) for k in range(4)], axis=1)
                res = jnp.dot(lhs, rhs, preferred_element_type=f32)
                if riders is not None:
                    next(riders, None)
            sink(i, _tile(res, i % m))
            if i % 2:
                for _ in range(min(2, len(late))):
                    mark(late.pop(0))
                for action in slow.pop(0) if slow else ():
                    action()
                if marked:
                    mark(_tile(res, i % m))
                pacer.run(2)

    def prep_heads(raw, row0, tmp, dst, g, scale, paced):
        for k in range(4):
            base = (g * 4 + k) * 64
            tmp[pl.ds(base, 64), :] = _as_u32(_as_bf16(raw[pl.ds(row0 + k * 64, 64), :]).T)
            for e in range(8):
                w = tmp[pl.ds(base + e, 8, stride=8), :]
                t = jnp.concatenate([_lo(w), _hi(w)], axis=0)
                if scale != 1.0:
                    t = t * scale
                t = _as_u32(t.astype(bf16))
                dst[k, _rows(g * 8 + e), :] = t
                if paced and e % 4 == 3:
                    mark_later(t, 8)
            yield 80

    def prep_wqkv(cps, raw, tmp, dst, scale):
        wait_here(cps, raw)
        for g in range(4):
            yield from prep_heads(raw, g * 256, tmp, dst, g, scale, True)

    def prep_wo():
        wait_here(cp_o, raw_o)
        for g in range(4):
            for k in range(4):
                ws = [raw_o[pl.ds(k * 256 + g * 64 + e, 8, stride=8), :] for e in range(8)]
                t = jnp.concatenate([f(w) for w in ws for f in (_lo, _hi)], axis=0)
                t = _as_u32(t.astype(bf16).T)
                wT_o[g, pl.ds(k * 64, 64), :] = t
                mark_later(t)
                yield 40

    def prep_router():
        wrt = jnp.broadcast_to(wr, (128, D)).T
        wrb[pl.ds(0, D), :] = wrt
        wrb[pl.ds(D, 8), :] = _bc(_colsum(wrt))
        later(lambda: mark(_tile(wrt, 63)))
        yield 128

    def slab(ref, t, k):
        return _as_bf16(ref[pl.ds(k * (FP // 2) + t * 64, 64), :])

    def prep_ffn(t):
        for raw, dst in ((raw_g, wg), (raw_u, wu)):
            for k in range(4):
                v = _as_u32(slab(raw, t, k).T)
                dst[t, pl.ds(k * 64, 64), :] = v
                mark_later(v)
                yield 24

    def layer_norm(key, tile, keep_at=None):
        s1, s2, res = _Acc(), _Acc(), []
        for i in range(64):
            res.append(tile(i))
            if keep_at is not None:
                xa0[keep_at, _rows(i), :] = res[i]
            if i == 0:
                shift = _shift(res[0])
                yield 28
                put(MA, _bc(shift))
            if i % 4 == 0:
                sb = get(MA)
            d = res[i] - sb
            s1.add(d)
            s2.add(d * d)
            if i % 4 == 3:
                yield 28
        dm, rstd = _moments(s1.tile(), s2.tile())
        rb = _bc(rstd)
        yield 40
        put(MA + 1, _bc(shift + dm))
        ts = []
        for i in range(64):
            if i % 8 == 0:
                mb = get(MA + 1)
            ts.append((res[i] - mb) * rb)
            if i % 8 == 7:
                yield 20
        xa[key] = lambda i: res[i]
        hv[key] = jnp.concatenate(ts, axis=0).astype(bf16)
        if keep_at is not None:
            h0[keep_at] = _as_u32(hv[key])

    def load_x(n):
        q = max(q for q, p in enumerate(PIECES) if p[0] <= n)
        if n == PIECES[q][0] and n:
            wait_here(cp_x[q], xs[q])
        return [_as_bf16(xs[q][pl.ds(k * 512 + n % 8, 64, stride=8), :]).T.astype(f32) for k in range(4)]

    def prep_input(n):
        ts = load_x(n)
        yield from layer_norm(n, lambda i: _tile(ts[i // 16], i % 16), n)

    def keep_input(n):
        for k, t in enumerate(load_x(n)):
            xb[n, pl.ds(k * 128, 128), :] = t
            later(lambda t=t: mark(_tile(t, 15)))
            yield 40

    def add_ln(n, paced=True):
        rstd = rs_s[pl.ds(n, 1), :]
        gain = [_bc(1.0 + rstd)]
        bias = _bc(m_s[pl.ds(n, 1), :] * rstd)

        def tile(i):
            if paced and i == 0:
                put(MA + 2, gain[0])
            if paced and i % 4 == 0:
                gain[0] = get(MA + 2)
            return xb[n, _rows(i), :] * gain[0] - bias
        return tile

    def prep(key, n, keep_at=None):
        yield from layer_norm(key, add_ln(n), keep_at)

    def q_mm(n, buf):
        pacer.until(lambda: n in hv)

        def sink(i, t):
            buf[QA + (n % 2) * 64 + i] = t
            q_ready.add((n, i))
        mm(wT_q, hv[n], sink, buf is not stage[0])

    def kv_first(w, key, ref, c, **kw):
        pacer.until(lambda: key in hv)

        def sink(i, t):
            ref[c + 8, _rows(i), :] = t
            ref[c, _rows(i), :] = pltpu.roll(t, 2, 1)
        mm(w, hv[key], sink, **kw)

    def kv_second(w, taps, prev, c):
        pacer.until(lambda: c + 8 in hv)

        def sink(i, t):
            taps[c + 8, i] = t
            if c > 0:
                taps[c, i] = pltpu.roll(jnp.where(lane >= 126, prev[c + 8, i], t), 2, 1)
        mm(w, hv[c + 8], sink)

    def attn(n, kt, vt):
        pend, outs = {}, []

        def flush(g):
            for w, p in enumerate(pend.pop(g, ())):
                put(PA + (g % 2) * 8 + w, p)

        def qk(g):
            ls = [None] * 8
            for d in range(16):
                while (n, g * 16 + d) not in q_ready:
                    yield 0
                qv = get(QA + (n % 2) * 64 + g * 16 + d)
                for w in range(8):
                    t = qv * kt[n % 8 + 8 - w, g * 16 + d]
                    ls[w] = ls[w] + t if d else t
                yield 15.5
            ls = [jnp.where(lane < 2, -1e9, ls[w]) if n < w else ls[w] for w in range(8)]
            top = _tree(ls, jnp.maximum)
            es = [jnp.exp(l - top) for l in ls]
            inv = 1.0 / _tree(es, jnp.add)
            pend[g] = [e * inv for e in es]
            later(lambda: flush(g), 5)
            yield 50

        def pv(g):
            flush(g)
            for half in range(2):
                acc = [None] * 8
                for w in range(8):
                    p = get(PA + (g % 2) * 8 + w)
                    for d in range(8):
                        t = p * vt[n % 8 + 8 - w, g * 16 + half * 8 + d]
                        acc[d] = acc[d] + t if w else t
                    yield 15.5
                outs.extend(acc)
                late.extend(acc)

        yield from qk(0)
        for g in range(4):
            if g < 3:
                yield from qk(g + 1)
            yield from pv(g)
        ov[n] = jnp.concatenate(outs, axis=0).astype(bf16)

    def keep_stats(n, shift, s1, s2, s3):
        dm, rstd = _moments(s1, s2)
        r_s[pl.ds(n, 1), :] = (_colsum(s3) - dm * wrb[pl.ds(D, 1), :]) * rstd
        m_s[pl.ds(n, 1), :] = shift[0:1] + dm
        rs_s[pl.ds(n, 1), :] = rstd

    def proj(n):
        pacer.until(lambda: n in ov)
        s1, s2, s3, shift = _Acc(), _Acc(), _Acc(), []

        def sink(i, t):
            t = xa[n](i) + t
            xb[n, _rows(i), :] = t
            if i == 0:
                shift.append(_bc(_shift(t)))
            d = t - shift[0]
            s1.add(d)
            s2.add(d * d)
            s3.add(d * wrb[_rows(i), :])
        mm(wT_o, ov[n], sink)
        return shift[0], s1.tile(), s2.tile(), s3.tile()

    def finish(n, paced=True):
        tile = add_ln(n, paced)
        q = max(q for q, p in enumerate(OUTS) if p[0] <= n)
        for k in range(4):
            ts = []
            for i in range(16):
                ts.append(tile(k * 16 + i))
                if i % 4 == 3:
                    yield 16
            t = _as_u32(jnp.concatenate(ts, axis=0).astype(bf16).T)
            xs[q][pl.ds(k * 512 + n % 8, 64, stride=8), :] = t
            if paced:
                mark_later(t)
        if n + 1 == sum(OUTS[q]):
            later(lambda: start_here(cp_out[q], xs[q]), DL + 2)

    def top2(nb):
        r = r_s[pl.ds(0, nb), :].astype(bf16).astype(f32)
        bits = _bits_u32(jnp.where(r == 0.0, 0.0, r)) >> 16
        u = jnp.where(bits >= 0x8000, u32(0xFFFF) - bits, bits + u32(0x8000))
        u = jnp.where(r != r, u32(0), u)
        rn = lax.broadcasted_iota(i32, (nb, 128), 0)
        rl = lax.broadcasted_iota(i32, (nb, 128), 1)
        pos = (rn >> 3) * 1024 + (rl >> 1) * 16 + (rn & 7) * 2 + (rl & 1)
        key = _bits_f32(u32(0x20000000) + (u << 11) + (S - 1 - pos).astype(u32))
        a1 = jnp.max(key, axis=0, keepdims=True)
        a2 = jnp.max(jnp.where(key == a1, 0.0, key), axis=0, keepdims=True)
        row = lax.broadcasted_iota(i32, (8, 128), 0)
        bit = (lane >> row) & 1
        za = jnp.max(jnp.where(row == 7, a1, jnp.where(bit == 0, a1, 0.0)), axis=1, keepdims=True)
        zb = jnp.max(jnp.where(row == 7, a2, jnp.where(bit == 1, a1, 0.0)), axis=1, keepdims=True)
        first = jnp.max(za, axis=0, keepdims=True)
        second = jnp.max(jnp.minimum(za, zb), axis=0, keepdims=True)
        kk = _bits_u32(jnp.where(row == 0, first, second)) - u32(0x20000000)
        uu = kk >> 11
        val = _bits_f32(jnp.where(uu >= 0x8000, uu - u32(0x8000), u32(0xFFFF) - uu) << 16)
        where = S - 1 - (kk & u32(S - 1)).astype(i32)
        sel = []
        for t in range(2):
            p = where[t, 0]
            sel.append((p, (p >> 10) * 8 + ((p >> 1) & 7), ((p >> 4) & 63) * 2 + (p & 1)))
        return sel, jax.nn.sigmoid(val)

    def ffn(sel, gate, out, pause, transposed):
        row = lax.broadcasted_iota(i32, (16, 128), 0)
        laned = lax.broadcasted_iota(i32, (D, 128), 1)
        picked = None
        for t, (_, n, l) in enumerate(sel):
            h = (xb[n] - m_s[pl.ds(n, 1), :]) * rs_s[pl.ds(n, 1), :]
            hb = jnp.where(laned == l, h, 0.0).astype(bf16)
            oh = jnp.where(row == t, 1.0, 0.0).astype(bf16)
            part = lax.dot_general(oh, hb, NT, preferred_element_type=f32)
            picked = part if picked is None else picked + part
            yield
        picked = picked.astype(bf16)
        for _ in range(pause):
            yield

        def wide(ref, t):
            return jnp.concatenate([slab(ref, t, k) for k in range(4)], axis=1)

        def up(raw, ready, t):
            if transposed:
                return jnp.dot(picked, _as_bf16(ready[t]), preferred_element_type=f32)
            return lax.dot_general(picked, wide(raw, t), NT, preferred_element_type=f32)
        acts = []
        for t in range(FP // 128):
            g_ = up(raw_g, wg, t)
            yield
            acts.append((g_ * jax.nn.sigmoid(g_) * up(raw_u, wu, t)).astype(bf16))
            yield
        y = None
        for t in range(FP // 128):
            part = jnp.dot(acts[t], wide(wd, t), preferred_element_type=f32)[0:8]
            y = part if y is None else y + part
            yield
        out.append(y * jnp.concatenate([gate()] * 4, axis=1))

    def scatter(sel, y):
        yb = _bits_u32(y.astype(bf16).astype(f32))
        yt = jnp.broadcast_to((yb[0:1] >> 16) | yb[1:2], (128, D)).T
        for t, (_, n, l) in enumerate(sel):
            tile = add_ln(n)
            for i in range(64):
                new = tile(i) + (_lo if t == 0 else _hi)(_tile(yt, i))
                pltpu.store(xb.at[n, _rows(i), :], new, mask=lane == l)
                if i % 4 == 3:
                    yield 20
            rs_s[pl.ds(n, 1), :] = jnp.where(lane[0:1] == l, 0.0, rs_s[pl.ds(n, 1), :])

    def patch_out(sel, y):
        row = lax.broadcasted_iota(i32, (8, 128), 0)
        cps = []
        for t, (p, _, _) in enumerate(sel):
            grp = p >> 4
            for k in range(4):
                at = pl.ds(pl.multiple_of(k * 512 + (grp & 63) * 8, 8), 8)
                w = jnp.where(row < 4, jnp.where(grp < 64, x0[at, :], x2[at, :]),
                              jnp.where(grp < 64, x1[at, :], jnp.where(row < 6, x3[at, :], x4[at, :])))
                halves = [_lo(w), _hi(w)]
                for t2, (p2, _, _) in enumerate(sel):
                    for odd in range(2):
                        halves[odd] = jnp.where(row * 2 + odd + grp * 16 == p2,
                                                halves[odd] + y[t2:t2 + 1, k * 128:(k + 1) * 128], halves[odd])
                even, odd = [_bits_u32(h.astype(bf16).astype(f32)) for h in halves]
                patch[_rows(t * 4 + k), :] = (even >> 16) | odd
            cps.append([pltpu.make_async_copy(
                patch.at[_rows(t * 4 + k)], out_hbm.bitcast(u32).at[grp, :, pl.ds(128 * k, 128)],
                sems.at[16 + t]) for k in range(4)])
        put(MA + 7, y[:, 0:128])
        for q in range(len(OUTS)):
            wait_here(cp_out[q], xs[q], 3)
        apart = (sel[0][0] >> 4) != (sel[1][0] >> 4)

        @pl.when(apart)
        def _():
            start(cps[0])
            start(cps[1])
            wait(cps[1])

        @pl.when(jnp.logical_not(apart))
        def _():
            start(cps[0])
        wait(cps[0])

    switch(st_a)
    m_s[pl.ds(8, 8), :] = jnp.zeros((8, 128), f32)
    rs_s[pl.ds(8, 8), :] = jnp.zeros((8, 128), f32)
    pacer.set([prep_input(0), prep_input(1)])

    def prep_wk(g):
        wait_here(cp_k[g:g + 1], raw_k[g])
        for _ in prep_heads(raw_k[g], 0, tmp_k, wT_k, g, 1.0, False):
            pass
    for g in range(2):
        for _ in range(10):
            pacer.step()
        prep_wk(g)
        mark(_bits_f32(raw_k[g][_rows(0), :]))
    pacer.drain()
    later(lambda: prep_wk(2), 0)
    later(lambda: prep_wk(3), 8)
    kv_first(wT_k, 0, k0, 0, m=32, tiles=range(32))
    pacer.set([prep_input(n) for n in range(2, 8)], 6 * PREP, 320)
    kv_first(wT_k, 1, k0, 1, m=32, tiles=range(32))
    for c in range(2):
        kv_first(wT_k, c, k0, c, m=32, tiles=range(32, 64))
    for c in range(2, 8):
        if c == 2:
            later(lambda: start_here(cp_q, raw_q), 2)
            later(lambda: start_here(cp_x[4], x4), 4)
            later(lambda: start_here(cp_o, raw_o), 40)
        kv_first(wT_k, c, k0, c)
        if c == 3:
            pacer.jobs.append(prep_wqkv(cp_v, raw_v, tmp_v, wT_v, 1.0))
    pacer.set([prep_wqkv(cp_q, raw_q, tmp_q, wT_q, 0.25), prep_router(), prep_input(8)]
              + [keep_input(n) for n in range(9, NB)] + [prep_wo()], WPREP + PREP + 1900, 500)
    for c in range(8):
        if c % 3 == 0:
            later(lambda c=c: start_here(*((cp_g, raw_g), (cp_u, raw_u), (cp_d, wd))[c // 3]), 2)
        kv_first(wT_v, c, v0, c)
    q_mm(0, st_b)
    settle()

    @pl.loop(0, 2)
    def _(layer):
        kt, vt = [{(e, i): ref[e, _rows(i), :] for e in range(1, 16) for i in range(64)} for ref in (k0, v0)]
        for i in range(64):
            first = _bc(vt[8, i][:, 0:1])
            for e in range(1, 8):
                vt[e, i] = jnp.where(lane < 2, first, vt[e, i])
        hv.clear()
        for n in range(9):
            hv[n] = _as_bf16(h0[n])
            xa[n] = lambda i, n=n: xa0[n, _rows(i), :]
        kt1, vt1, order = {}, {}, []
        switch(st_b)
        for c in range(8):
            pacer.set(([prep(c + 9, c + 9)] if c < 7 else []) + [attn(c, kt, vt)], PREP + ATT, 192)
            kv_second(wT_k, kt1, kt, c)
            kv_second(wT_v, vt1, vt, c)
            q_mm(c + 1, st_b if c < 7 else st_c)
        switch(st_c)
        pacer.set([attn(n, kt1, vt1) for n in range(8, NB)], 8 * ATT + 14 * FIN + PREP, 21.5 * 64)
        for step in PLAN.split():
            n = int(step[1:])
            if step[0] == "q":
                pacer.until(lambda: n - 2 in ov)
                q_mm(n, st_c)
                continue
            keep_stats(n, *proj(n))
            if n == 12:
                pacer.urgent.append(prep(NB, order[0], order[0]))
            pacer.urgent.append(finish(n))
            if n == 11:
                cand, _ = top2(8)
                ca, cb = cand[0][1] & 7, cand[1][1] & 7
                cb = jnp.where(ca == cb, (ca + 1) & 7, cb)
                lo, hi = jnp.minimum(ca, cb), jnp.maximum(ca, cb)
                for s in range(6):
                    c = s + (s >= lo).astype(i32)
                    order.append(c + (c >= hi).astype(i32))
                order.extend([lo, hi])
        for i, t in enumerate(proj(15)):
            sums[i] = t
        settle()

        @pl.when(layer == 0)
        def _():
            switch(st_a)
            keep_stats(15, *[sums[i] for i in range(4)])
            sel, gate = top2(NB)
            for cps in (cp_g, cp_u, cp_d):
                wait(cps)
            for q in range(len(OUTS) - 1):
                later(lambda q=q: wait_here(cp_out[q], xs[q], 3), 200)
            hv.clear()
            hv[NB] = _as_bf16(h0[order[0]])
            y = []
            riders = ffn(sel, lambda: gate, y, 2, False)
            for s in range(8):
                if s != 5:
                    nxt = prep(NB + s + 1, order[s + 1], order[s + 1]) if s < 7 else prep(8, 8, 8)
                    extra = [prep_ffn(t) for t in {6: range(6), 7: range(6, 11)}.get(s, ())]
                    pacer.set([nxt] + extra, PREP + 192 * len(extra), 128 if extra else 60 if s == 4 else 80)
                m = {1: 16, 2: 16, 3: 16, 4: 8}.get(s)
                kv_first(wT_k, NB + s, k0, order[s], **(dict(riders=riders, m=m) if m else {}))
                if s == 4:
                    pacer.set([scatter(sel, y[0]), prep(NB + 6, order[6], order[6])], PREP + 640, 150)
                m = {0: 16, 1: 16, 2: 16, 3: 8}.get(s)
                kv_first(wT_v, NB + s, v0, order[s], **(dict(riders=riders, m=m) if m else {}))
            pacer.drain()
            hv[0] = _as_bf16(h0[0])
            q_mm(0, st_b)
            settle()

    switch(st_a)
    keep_stats(15, *[sums[i] for i in range(4)])
    sel, gate = top2(NB)
    y = []
    riders = ffn(sel, lambda: get(MA), y, 0, True)
    next(riders)
    next(riders)
    pacer.set([finish(15, False)])
    settle()
    put(MA, gate)
    for _ in riders:
        pass
    patch_out(sel, y[0])


@jax.jit
def pallas_interleave_layers__sliding_local_dilated__moe_arch_mod__prompt_kernel(
        A_x, A_wqkv, A_wo, B_x, B_w_r, B_w_gate, B_w_up, B_w_down):
    del B_x
    hbm = pl.BlockSpec(memory_space=pltpu.MemorySpace.HBM)
    vm = pltpu.VMEM
    out = pl.pallas_call(
        kernel,
        grid=(1,),
        out_shape=jax.ShapeDtypeStruct((S // 16, 16, D), bf16),
        in_specs=[hbm] * 7,
        out_specs=hbm,
        scratch_shapes=(
            [vm((4 * 512 + SPARE, 128), u32)] * 5
            + [vm((256 + SPARE, 128), u32)] * 4
            + [vm((4 * 256 + SPARE, 128), u32)] * 6
            + [vm((4, D // 2, 128), u32)] * 4
            + [vm((NB, D, 128), f32)] * 3
            + [vm((9, D, 128), f32)]
            + [vm((9, D // 2, 128), u32)]
            + [vm((NB, 128), f32)] * 3
            + [vm((4, 8, 128), f32)]
            + [vm((4 * FP // 2 + SPARE, 128), u32)] * 3
            + [vm((FP // 128, D // 2, 128), u32)] * 2
            + [vm((D,), bf16), vm((D + 8, 128), f32)]
            + [vm((64, 128), u32)]
            + [vm((SLOTS, 8, 128), f32)] * 3
            + [pltpu.SemaphoreType.DMA((18,))]
        ),
        compiler_params=pltpu.CompilerParams(
            vmem_limit_bytes=120 * 1024 * 1024,
            flags={"XLA_TPU_RESCHEDULE_DMA_DONES": True},
            disable_bounds_checks=True, disable_semaphore_checks=True),
    )(A_x.reshape(S // 16, 16, D), A_wqkv, A_wo, B_w_r, B_w_gate.T, B_w_up.T, B_w_down)
    return out.reshape(1, S, D)
```
